```python
import os as _os
_os.environ.setdefault("JAX_PLATFORMS", "cpu")
import jax
import jax.numpy as jnp

def _softmax(x, axis=-1):
    return jax.nn.softmax(x, axis=axis)
def _gelu(x):
    return jax.nn.gelu(x, approximate=True)
def _silu(x):
    return jax.nn.silu(x)
def _sigmoid(x):
    return jax.nn.sigmoid(x)
def _layernorm(x, axis=-1, eps=1e-5):
    m = jnp.mean(x, axis=axis, keepdims=True)
    v = jnp.var(x, axis=axis, keepdims=True)
    return (x - m) / jnp.sqrt(v + eps)
def _scatter_add(tgt, idx, src, axis=0):
    return tgt.at[idx].add(src)
def _segment_sum(src, seg, n):
    return jax.ops.segment_sum(src, seg, n)
class _Rng:
    def __init__(self, key):
        self._k = key
    def _next(self):
        self._k, sub = jax.random.split(self._k)
        return sub
    def normal(self, shape):
        return jax.random.normal(self._next(), shape, dtype=jnp.bfloat16)
    def randint(self, lo, hi, shape):
        return jax.random.randint(self._next(), shape, lo, hi, dtype=jnp.int32)
    def uniform(self, shape, lo=0.0, hi=1.0):
        return jax.random.uniform(self._next(), shape, jnp.bfloat16, lo, hi)
    def permutation(self, n):
        return jax.random.permutation(self._next(), n)


kernel_name = 'parallel_sum__spectral_gfnet__glu_gated_swiglu__prompt'

def setup_inputs():
    _rng = _Rng(jax.random.key(int.from_bytes(__import__("os").urandom(4), "little")))
    _w = (lambda a: (lambda t: t.astype(jnp.bfloat16) if jnp.issubdtype(t.dtype, jnp.floating) else t)(jnp.asarray(a)))
    def _A_setup():
        B, S, D = 1, 2048, 512
        Df = D // 2 + 1
        return {
            "x": _w((lambda *s: _rng.normal(s) * 0.05)(B, S, D)),
            "w_r": _w((lambda *s: _rng.normal(s) * 0.2)(S, Df) * 0.02),
            "w_i": _w((lambda *s: _rng.normal(s) * 0.2)(S, Df) * 0.02),
        }
    _A_in = _A_setup()

    def _B_setup():
        B, S, D, F = 1, 2048, 512, 1376
        return {
            "x": _w((lambda *s: _rng.normal(s) * 0.05)(B, S, D)),
            "w1": _w((lambda *s: _rng.normal(s) * 0.05)(D, F) * (2.0 / D) ** 0.5),
            "w3": _w((lambda *s: _rng.normal(s) * 0.05)(D, F) * (2.0 / D) ** 0.5),
            "w2": _w((lambda *s: _rng.normal(s) * 0.05)(F, D) * (2.0 / F) ** 0.5),
        }
    _B_in = _B_setup()

    return {
        "A_x": _A_in["x"],
        "A_w_r": _A_in["w_r"],
        "A_w_i": _A_in["w_i"],
        "B_x": _B_in["x"],
        "B_w1": _B_in["w1"],
        "B_w3": _B_in["w3"],
        "B_w2": _B_in["w2"],
    }

def reference(A_x, A_w_r, A_w_i, B_x, B_w1, B_w3, B_w2):
    def _A_ref(x, w_r, w_i):
        B, S, D = x.shape
        X = (lambda x, axes=(-2,-1): jnp.fft.rfft2(x.astype(jnp.float32), axes=axes))(x, axes=(-2, -1))
        W = w_r + 1j * w_i
        X = X * W
        y = (lambda x, s, axes=(-2,-1): jnp.fft.irfft2(x, s=s, axes=axes).astype(jnp.bfloat16))(X, (S, D), axes=(-2, -1))
        return y

    def _B_ref(x, w1, w3, w2):
        gate = jnp.einsum("bsd,df->bsf", x, w1)
        up = jnp.einsum("bsd,df->bsf", x, w3)
        h = _silu(gate) * up
        out = jnp.einsum("bsf,fd->bsd", h, w2)
        return out

    x = A_x
    xn = _layernorm(x, axis=-1)
    return x + _A_ref(xn, A_w_r, A_w_i) + _B_ref(xn, B_w1, B_w3, B_w2)
```

```python
import jax
import jax.numpy as jnp
import numpy as np
import jax.experimental.pallas as pl
import jax.experimental.pallas.tpu as pltpu

S, D, F, T = 2048, 512, 1376, 256
BF, F32 = jnp.bfloat16, jnp.float32


def _consts():
    d = np.arange(D)[:, None]; l = np.arange(256)[None]
    a = 2 * np.pi * d * l / D
    fd = np.concatenate([np.cos(a), -np.sin(a)], 1)
    sc = np.where(l == 0, 1.0, 2.0)
    gi = (-np.sin(a) * sc).T.copy()
    gi[0] = (-1.0) ** np.arange(D)
    gd = np.concatenate([(np.cos(a) * sc).T, gi], 0) / D
    k2 = np.arange(128)[:, None]; n2 = np.arange(128)[None]
    fs = []
    for k1 in range(16):
        m = np.exp(-2j * np.pi * n2 * (k1 + 16 * k2) / S)
        fs.append(np.block([[m.real, -m.imag], [m.imag, m.real]]))
    fs = np.stack(fs)
    f16 = np.zeros((128, 128), complex)
    f16[:16, :16] = np.exp(-2j * np.pi * np.outer(np.arange(16), np.arange(16)) / 16)
    tw = np.zeros((128, 128), complex)
    tw[:, :16] = np.exp(-2j * np.pi * np.arange(128)[:, None] * np.arange(16)[None] / S)
    m = np.block([[f16.real, f16.imag], [-f16.imag, f16.real]])
    return (fd, gd, fs, fs.transpose(0, 2, 1), m, np.stack([tw.real, tw.imag]))


_C = _consts()


def _fft(v, sign):
    n = len(v)
    if n == 1:
        return v
    e, o = _fft(v[0::2], sign), _fft(v[1::2], sign)
    out = [None] * n
    for k in range(n // 2):
        r, i = o[k]
        if k == 0:
            tr, ti = r, i
        elif 4 * k == n:
            tr, ti = (i, -r) if sign < 0 else (-i, r)
        else:
            c = float(np.cos(2 * np.pi * k / n)); s = float(sign * np.sin(2 * np.pi * k / n))
            tr, ti = r * c - i * s, r * s + i * c
        out[k] = (e[k][0] + tr, e[k][1] + ti)
        out[k + n // 2] = (e[k][0] - tr, e[k][1] - ti)
    return out


def _dot(a, b):
    return jnp.dot(a.astype(BF), b.astype(BF), preferred_element_type=F32)


def _kernel(x_ref, r0, r1, r2, i0, i1, i2, w1h, w3h, w2h, fd, gd, fs, fst, m16, tw, o_ref,
            w1, w3, w2, sem, xn_s, z, acc, cn, wn, wf):
    g = pl.program_id(0)
    cps = [pltpu.make_async_copy(a, b, sem.at[i])
           for i, (a, b) in enumerate(((w1h, w1), (w3h, w3), (w2h, w2)))]
    lane = jax.lax.broadcasted_iota(jnp.int32, (128, 128), 1)

    @pl.when(g == 0)
    def _():
        for c in cps:
            c.start()
        cn[...] = jnp.zeros_like(cn)
        wn[...] = jnp.zeros_like(wn)

    @pl.when(g < 8)
    def _():
        x = x_ref[...].astype(F32)
        m = jnp.mean(x, -1, keepdims=True)
        xc = x - m
        v = jnp.mean(xc * xc, -1, keepdims=True)
        xn = (xc * jax.lax.rsqrt(v + 1e-5)).astype(BF)
        r = pl.ds(pl.multiple_of(g * T, T), T)
        xn_s[r, :] = xn
        acc[r, :] = x
        for q, f in enumerate((r0, r1, r2, i0, i1, i2)):
            wf[q, r, :] = f[...].astype(F32)
        z[r, :] = jnp.dot(xn, fd[...], preferred_element_type=F32)
        sg = (1 - 2 * (jax.lax.broadcasted_iota(jnp.int32, (1, D), 1) & 1)).astype(F32)
        c = jnp.sum(xn.astype(F32) * sg, -1, keepdims=True)
        cn[0] = jnp.where(lane == 2 * g, c[:128], jnp.where(lane == 2 * g + 1, c[128:], cn[0]))

    def radix(sign):
        def body(t, _):
            for cb in range(2):
                v = []
                for n in range(16):
                    r = pl.ds(pl.multiple_of(n * 128 + t * 8, 8), 8)
                    v.append((z[r, cb * 128:cb * 128 + 128], z[r, 256 + cb * 128:384 + cb * 128]))
                v = _fft(v, sign)
                for n in range(16):
                    r = pl.ds(pl.multiple_of(n * 128 + t * 8, 8), 8)
                    z[r, cb * 128:cb * 128 + 128] = v[n][0]
                    z[r, 256 + cb * 128:384 + cb * 128] = v[n][1]
        jax.lax.fori_loop(0, 16, body, None)

    @pl.when(g == 8)
    def _():
        radix(-1)
        for c in cps:
            c.wait()

    @pl.when(jnp.logical_and(g > 8, g < 17))
    def _():
        j = g - 9
        for p in range(2):
            k1 = 2 * j + p
            r = pl.ds(pl.multiple_of(k1 * 128, 128), 128)
            zz = jnp.concatenate([z[r, :256], z[r, 256:]], 0)
            y = _dot(fs[p], zz)
            a, b = (jnp.concatenate([wf[3 * q + c, pl.ds(k1, 128, stride=16), :] for c in range(3)], 1)
                    for q in range(2))
            for q, w in enumerate((a, b)):
                wn[q] = jnp.where(lane == k1, w[:, 256:257], wn[q])
            a, b = a[:, :256] * (1.0 / S), b[:, :256] * (1.0 / S)
            yr, yi = y[:128], y[128:]
            y = _dot(fst[p], jnp.concatenate([yr * a - yi * b, yr * b + yi * a], 0))
            z[r, :256] = y[:128]
            z[r, 256:] = y[128:]
        r = pl.ds(pl.multiple_of(j * T, T), T)
        xn = xn_s[r, :]
        ga = jnp.dot(xn, w1[...], preferred_element_type=F32)
        up = jnp.dot(xn, w3[...], preferred_element_type=F32)
        h = ga * jax.nn.sigmoid(ga) * up
        acc[r, :] += jnp.dot(h.astype(BF), w2[...], preferred_element_type=F32)

    @pl.when(g == 17)
    def _():
        radix(1)
        t = _dot(cn[0], m16[:128, :])
        a, b = t[:, :128], t[:, 128:]
        c, s = tw[0], tw[1]
        y = _dot(fs[0], jnp.concatenate([a * c - b * s, a * s + b * c], 0))
        a, b = y[:128], y[128:]
        p, q = wn[0] * (1.0 / S), wn[1] * (1.0 / S)
        y = _dot(fst[0], jnp.concatenate([a * p - b * q, a * q + b * p], 0))
        a, b = y[:128], y[128:]
        u = jnp.concatenate([a * c + b * s, a * s - b * c], 1)
        cn[0] = _dot(u, m16[:, :128])

    @pl.when(g > 17)
    def _():
        j = g - 18
        r = pl.ds(pl.multiple_of(j * T, T), T)
        c = cn[0]
        c = jnp.concatenate([jnp.sum(jnp.where(lane == 2 * j + p, c, 0.0), -1, keepdims=True)
                             for p in range(2)], 0)
        zz = z[r, :]
        zz = jnp.where(jax.lax.broadcasted_iota(jnp.int32, (T, D), 1) == 256, c, zz)
        o_ref[...] = (acc[r, :] + _dot(zz, gd[...])).astype(BF)


@jax.jit
def pallas_parallel_sum__spectral_gfnet__glu_gated_swiglu__prompt_kernel(
        A_x, A_w_r, A_w_i, B_x, B_w1, B_w3, B_w2):
    cs = [jnp.asarray(c.astype(np.float32).astype(BF)) for c in _C[:5]] + [jnp.asarray(_C[5].astype(np.float32))]
    full = lambda s: pl.BlockSpec(s, lambda g: (0,) * len(s))
    fsp = pl.BlockSpec((2, 256, 256), lambda g: (jnp.where(g < 17, jnp.clip(g - 9, 0, 7), 0), 0, 0))
    anys = pl.BlockSpec(memory_space=pl.ANY)
    out = pl.pallas_call(
        _kernel, grid=(26,),
        in_specs=[pl.BlockSpec((T, D), lambda g: (jnp.minimum(g, 7), 0)),
                  *[pl.BlockSpec((T, 128), lambda g, c=c: (jnp.minimum(g, 7), c)) for c in (0, 1, 2) * 2], anys, anys, anys,
                  full((D, D)), full((D, D)), fsp, fsp, full((256, 256)), full((2, 128, 128))],
        out_specs=pl.BlockSpec((T, D), lambda g: (jnp.maximum(g - 18, 0), 0)),
        out_shape=jax.ShapeDtypeStruct((S, D), BF),
        scratch_shapes=[pltpu.VMEM((D, F), BF), pltpu.VMEM((D, F), BF), pltpu.VMEM((F, D), BF),
                        pltpu.SemaphoreType.DMA((3,)), pltpu.VMEM((S, D), BF), pltpu.VMEM((S, D), F32),
                        pltpu.VMEM((S, D), F32), pltpu.VMEM((1, 128, 128), F32), pltpu.VMEM((2, 128, 128), F32),
                        pltpu.VMEM((6, S, 128), F32)],
        compiler_params=pltpu.CompilerParams(dimension_semantics=("arbitrary",), vmem_limit_bytes=100 << 20),
    )(A_x.reshape(S, D), *[A_w_r] * 3, *[A_w_i] * 3, B_w1, B_w3, B_w2, *cs)
    return out.reshape(1, S, D)
```
